```python
import os as _os
_os.environ.setdefault("JAX_PLATFORMS", "cpu")
import jax
import jax.numpy as jnp

def _softmax(x, axis=-1):
    return jax.nn.softmax(x, axis=axis)
def _gelu(x):
    return jax.nn.gelu(x, approximate=True)
def _silu(x):
    return jax.nn.silu(x)
def _sigmoid(x):
    return jax.nn.sigmoid(x)
def _layernorm(x, axis=-1, eps=1e-5):
    m = jnp.mean(x, axis=axis, keepdims=True)
    v = jnp.var(x, axis=axis, keepdims=True)
    return (x - m) / jnp.sqrt(v + eps)
def _scatter_add(tgt, idx, src, axis=0):
    return tgt.at[idx].add(src)
def _segment_sum(src, seg, n):
    return jax.ops.segment_sum(src, seg, n)
class _Rng:
    def __init__(self, key):
        self._k = key
    def _next(self):
        self._k, sub = jax.random.split(self._k)
        return sub
    def normal(self, shape):
        return jax.random.normal(self._next(), shape, dtype=jnp.bfloat16)
    def randint(self, lo, hi, shape):
        return jax.random.randint(self._next(), shape, lo, hi, dtype=jnp.int32)
    def uniform(self, shape, lo=0.0, hi=1.0):
        return jax.random.uniform(self._next(), shape, jnp.bfloat16, lo, hi)
    def permutation(self, n):
        return jax.random.permutation(self._next(), n)


kernel_name = 'interleave_layers__linear_kernel_hedgehog__dense_activation_silu__prompt'

def setup_inputs():
    _rng = _Rng(jax.random.key(int.from_bytes(__import__("os").urandom(4), "little")))
    _w = (lambda a: (lambda t: t.astype(jnp.bfloat16) if jnp.issubdtype(t.dtype, jnp.floating) else t)(jnp.asarray(a)))
    def _A_setup():
        B, S, D, H = 1, 2048, 640, 32
        Dh = D // H
        return {
            "x": _w((lambda *s: _rng.normal(s) * 0.05)(B, S, D)),
            "wqkv": _w((lambda *s: _rng.normal(s) * 0.4)(D, 3 * D)),
            "w_phi": _w((lambda *s: _rng.normal(s) * 0.4)(H, Dh, Dh) * (Dh ** -0.5)),
            "wo": _w((lambda *s: _rng.normal(s) * 0.05)(D, D)),
        }
    _A_in = _A_setup()

    def _B_setup():
        B, S, D, F = 1, 2048, 640, 1728
        return {
            "x": _w((lambda *s: _rng.normal(s) * 0.05)(B, S, D)),
            "w1": _w((lambda *s: _rng.normal(s) * 1.6)(D, F) * (D ** -0.5)),
            "w2": _w((lambda *s: _rng.normal(s) * 1.6)(F, D) * (F ** -0.5)),
        }
    _B_in = _B_setup()

    return {
        "A_x": _A_in["x"],
        "A_wqkv": _A_in["wqkv"],
        "A_w_phi": _A_in["w_phi"],
        "A_wo": _A_in["wo"],
        "B_x": _B_in["x"],
        "B_w1": _B_in["w1"],
        "B_w2": _B_in["w2"],
    }

def reference(A_x, A_wqkv, A_w_phi, A_wo, B_x, B_w1, B_w2):
    def _A_ref(x, wqkv, w_phi, wo):
        B, S, D = x.shape
        H = 32; Dh = D // H
        qkv = (lambda x, *d: x.transpose(*d))((x @ wqkv).reshape(B, S, 3, H, Dh), 2, 0, 3, 1, 4)
        q, k, v = qkv[0], qkv[1], qkv[2]
        pq = jnp.einsum("bhsd,hdf->bhsf", q, w_phi)
        pk = jnp.einsum("bhsd,hdf->bhsf", k, w_phi)
        phi_q = jnp.concatenate([_softmax(pq, axis=-1), _softmax(-pq, axis=-1)], axis=-1)
        phi_k = jnp.concatenate([_softmax(pk, axis=-1), _softmax(-pk, axis=-1)], axis=-1)
        kv = jnp.einsum("bhsf,bhsd->bhfd", phi_k, v)
        z  = jnp.einsum("bhsf->bhf", phi_k)
        num = jnp.einsum("bhqf,bhfd->bhqd", phi_q, kv)
        den = jnp.einsum("bhqf,bhf->bhq", phi_q, z)[..., None] + 1e-6
        o = num / den
        return (lambda x, *d: x.transpose(*d))(o, 0, 2, 1, 3).reshape(B, S, D) @ wo

    def _B_ref(x, w1, w2):
        h = jnp.einsum("bsd,df->bsf", x, w1)
        h = _silu(h)
        out = jnp.einsum("bsf,fd->bsd", h, w2)
        return out

    x = A_x
    x = x + _A_ref(_layernorm(x, axis=-1), A_wqkv, A_w_phi, A_wo)
    x = x + _B_ref(_layernorm(x, axis=-1), B_w1, B_w2)
    x = x + _A_ref(_layernorm(x, axis=-1), A_wqkv, A_w_phi, A_wo)
    x = x + _B_ref(_layernorm(x, axis=-1), B_w1, B_w2)
    return x
```

```python
import jax
import jax.numpy as jnp
from jax import lax
from jax.experimental import pallas as pl
from jax.experimental.pallas import tpu as pltpu

S = 2048
D = 640
H = 32
DH = 20
F = 1728
NG = 4
L = 8
GW = DH * L
PHI_ROWS = 384
V_ROWS = 176
T = 512
NT_TILES = S // T

_NN = (((1,), (0,)), ((), ()))
_NT = (((1,), (1,)), ((), ()))
_TN = (((0,), (0,)), ((), ()))


def _dot(a, b, dn):
    return lax.dot_general(a, b, dn, preferred_element_type=jnp.float32)


def _layernorm_bf16(x):
    m = jnp.mean(x, axis=-1, keepdims=True)
    xc = x - m
    v = jnp.mean(xc * xc, axis=-1, keepdims=True)
    return (xc * lax.rsqrt(v + 1e-5)).astype(jnp.bfloat16)


def _hedgehog_features(p):
    t = p.shape[-1]
    p = p.reshape(NG, DH, L, t)
    mx = jnp.max(p, axis=1, keepdims=True)
    mn = jnp.min(p, axis=1, keepdims=True)
    ep = jnp.exp(p - mx)
    em = jnp.exp(mn - p)
    sp = jnp.sum(ep, axis=1, keepdims=True)
    sm = jnp.sum(em, axis=1, keepdims=True)
    phi = jnp.concatenate([ep * (1.0 / sp), em * (1.0 / sm)], axis=1)
    return phi.reshape(NG, 2 * GW, t).astype(jnp.bfloat16)


def _kernel(x_hbm, wqkv_hbm, wphi_ref, wo_hbm, w1t_hbm, w2_hbm, o_ref,
            xs_ref, wt_ref, wop_ref, phiq_ref, phik_ref, vt_ref, kvt_ref,
            x_ref, wqkv_ref, wo_ref, w1t_ref, w2_ref, sems):
    copies = [
        pltpu.make_async_copy(wqkv_hbm, wqkv_ref, sems.at[0]),
        pltpu.make_async_copy(x_hbm, x_ref, sems.at[1]),
        pltpu.make_async_copy(wo_hbm, wo_ref, sems.at[2]),
        pltpu.make_async_copy(w1t_hbm, w1t_ref, sems.at[3]),
        pltpu.make_async_copy(w2_hbm, w2_ref, sems.at[4]),
    ]
    for c in copies:
        c.start()

    row = lax.broadcasted_iota(jnp.int32, (D, D), 0)
    col = lax.broadcasted_iota(jnp.int32, (D, D), 1)
    row_head = (row // GW) * L + row % L
    row_idx = (row % GW) // L
    perm = (col == row_head * DH + row_idx).astype(jnp.bfloat16)

    r128 = lax.broadcasted_iota(jnp.int32, (D, 128), 0)
    c128 = lax.broadcasted_iota(jnp.int32, (D, 128), 1)
    sel_f = (c128 == (r128 % GW) // L).astype(jnp.bfloat16)
    gfull = _dot(sel_f, wphi_ref[...], _NT)
    gt = jnp.where(col // DH == row_head, gfull, 0.0).astype(jnp.bfloat16)

    copies[0].wait()

    wt_ref[0:D, :] = _dot(gt, wqkv_ref[:, 0:D], _NT).astype(jnp.bfloat16)
    wt_ref[D:2 * D, :] = _dot(gt, wqkv_ref[:, D:2 * D], _NT).astype(jnp.bfloat16)
    wt_ref[2 * D:3 * D, :] = _dot(perm, wqkv_ref[:, 2 * D:3 * D], _NT).astype(jnp.bfloat16)
    copies[1].wait()
    xs_ref[...] = x_ref[...].astype(jnp.float32)

    zpad = jnp.zeros((PHI_ROWS - 2 * GW, S), jnp.bfloat16)
    ones_rows = jnp.concatenate(
        [jnp.ones((L, S), jnp.bfloat16), jnp.zeros((V_ROWS - GW - L, S), jnp.bfloat16)], axis=0)
    for g in range(NG):
        phiq_ref[g, 2 * GW:PHI_ROWS, :] = zpad
        phik_ref[g, 2 * GW:PHI_ROWS, :] = zpad
        vt_ref[g, GW:V_ROWS, :] = ones_rows

    def a_phase1(i, carry):
        t0 = pl.multiple_of(i * T, T)
        xn = _layernorm_bf16(xs_ref[pl.ds(t0, T), :])
        pv = _dot(wt_ref[...], xn, _NT)
        phiq = _hedgehog_features(pv[0:D])
        phik = _hedgehog_features(pv[D:2 * D])
        vt = pv[2 * D:3 * D].reshape(NG, GW, T).astype(jnp.bfloat16)
        for g in range(NG):
            phiq_ref[g, 0:2 * GW, pl.ds(t0, T)] = phiq[g]
            phik_ref[g, 0:2 * GW, pl.ds(t0, T)] = phik[g]
            vt_ref[g, 0:GW, pl.ds(t0, T)] = vt[g]
        return carry

    def a_state():
        r = lax.broadcasted_iota(jnp.int32, (V_ROWS, PHI_ROWS), 0)
        c = lax.broadcasted_iota(jnp.int32, (V_ROWS, PHI_ROWS), 1)
        same_head = (r % L) == (c % L)
        for g in range(NG):
            kv = _dot(vt_ref[g], phik_ref[g], _NT)
            kvt_ref[g] = jnp.where(same_head, kv, 0.0).astype(jnp.bfloat16)

    def a_phase2(i, carry):
        t0 = pl.multiple_of(i * T, T)
        outs = []
        for g in range(NG):
            nd = _dot(kvt_ref[g], phiq_ref[g, :, pl.ds(t0, T)], _NN)
            inv = 1.0 / (nd[GW:GW + L] + 1e-6)
            o = nd[0:GW].reshape(DH, L, T) * inv[None]
            outs.append(o.reshape(GW, T).astype(jnp.bfloat16))
        ot = jnp.concatenate(outs, axis=0)
        attn = _dot(ot, wop_ref[...], _TN)
        xs_ref[pl.ds(t0, T), :] += attn
        return carry

    def b_layer(i, carry):
        t0 = pl.multiple_of(i * T, T)
        x = xs_ref[pl.ds(t0, T), :]
        xn = _layernorm_bf16(x)
        h = _dot(xn, w1t_ref[...], _NT)
        h = (h * jax.nn.sigmoid(h)).astype(jnp.bfloat16)
        y = _dot(h, w2_ref[...], _NN)
        xs_ref[pl.ds(t0, T), :] = x + y
        return carry

    for layer in range(2):
        lax.fori_loop(0, NT_TILES, a_phase1, 0)
        a_state()
        if layer == 0:
            copies[2].wait()
            wop_ref[...] = _dot(perm, wo_ref[...], _NN).astype(jnp.bfloat16)
        lax.fori_loop(0, NT_TILES, a_phase2, 0)
        if layer == 0:
            copies[3].wait()
            copies[4].wait()
        lax.fori_loop(0, NT_TILES, b_layer, 0)

    o_ref[...] = xs_ref[...].astype(o_ref.dtype)


@jax.jit
def pallas_interleave_layers__linear_kernel_hedgehog__dense_activation_silu__prompt_kernel(
    A_x: jax.Array,
    A_wqkv: jax.Array,
    A_w_phi: jax.Array,
    A_wo: jax.Array,
    B_x: jax.Array,
    B_w1: jax.Array,
    B_w2: jax.Array,
):
    del B_x
    x = A_x.reshape(S, D)
    wphi = jnp.pad(A_w_phi.reshape(H * DH, DH), ((0, 0), (0, 128 - DH)))

    out = pl.pallas_call(
        _kernel,
        out_shape=jax.ShapeDtypeStruct((S, D), A_x.dtype),
        in_specs=[
            pl.BlockSpec(memory_space=pl.ANY),
            pl.BlockSpec(memory_space=pl.ANY),
            pl.BlockSpec(memory_space=pltpu.VMEM),
            pl.BlockSpec(memory_space=pl.ANY),
            pl.BlockSpec(memory_space=pl.ANY),
            pl.BlockSpec(memory_space=pl.ANY),
        ],
        scratch_shapes=[
            pltpu.VMEM((S, D), jnp.float32),
            pltpu.VMEM((3 * D, D), jnp.bfloat16),
            pltpu.VMEM((D, D), jnp.bfloat16),
            pltpu.VMEM((NG, PHI_ROWS, S), jnp.bfloat16),
            pltpu.VMEM((NG, PHI_ROWS, S), jnp.bfloat16),
            pltpu.VMEM((NG, V_ROWS, S), jnp.bfloat16),
            pltpu.VMEM((NG, V_ROWS, PHI_ROWS), jnp.bfloat16),
            pltpu.VMEM((S, D), jnp.bfloat16),
            pltpu.VMEM((D, 3 * D), jnp.bfloat16),
            pltpu.VMEM((D, D), jnp.bfloat16),
            pltpu.VMEM((F, D), jnp.bfloat16),
            pltpu.VMEM((F, D), jnp.bfloat16),
            pltpu.SemaphoreType.DMA((5,)),
        ],
        compiler_params=pltpu.CompilerParams(vmem_limit_bytes=100 * 1024 * 1024),
    )(x, A_wqkv, wphi, A_wo, B_w1.T, B_w2)
    return out.reshape(1, S, D)
```

```python
import jax
import jax.numpy as jnp
from jax import lax
from jax.experimental import pallas as pl
from jax.experimental.pallas import tpu as pltpu

S = 2048
D = 640
H = 32
DH = 20
F = 1728
NG = 4
L = 8
GW = DH * L
PHI_ROWS = 384
V_ROWS = 176
WIN = 256
T = 1024
NT_TILES = S // T
TB = 1024
NB_TILES = S // TB
assert S % T == 0 and S % TB == 0 and NT_TILES >= 2 and NB_TILES >= 2 and TB <= T

_NN = (((1,), (0,)), ((), ()))
_NT = (((1,), (1,)), ((), ()))
_TN = (((0,), (0,)), ((), ()))


def _dot(a, b, dn):
    return lax.dot_general(a, b, dn, preferred_element_type=jnp.float32)


def _layernorm_bf16(x):
    m = jnp.mean(x, axis=-1, keepdims=True)
    xc = x - m
    v = jnp.mean(xc * xc, axis=-1, keepdims=True)
    return (xc * lax.rsqrt(v + 1e-5)).astype(jnp.bfloat16)


def _hedgehog_features(p):
    t = p.shape[-1]
    p = p.reshape(NG, DH, L, t)
    mx = jnp.max(p, axis=1, keepdims=True)
    mn = jnp.min(p, axis=1, keepdims=True)
    ep = jnp.exp(p - mx)
    em = jnp.exp(mn - p)
    sp = jnp.sum(ep, axis=1, keepdims=True)
    sm = jnp.sum(em, axis=1, keepdims=True)
    phi = jnp.concatenate([ep * (1.0 / sp), em * (1.0 / sm)], axis=1)
    return phi.reshape(NG, 2 * GW, t).astype(jnp.bfloat16)


def _win0(g):
    return (g * GW) // 128 * 128


def _kernel(x_hbm, wqkv_hbm, wphi_ref, wo_hbm, w1t_hbm, w2_hbm, o_hbm,
            xs_ref, wt_ref, wop_ref, phiq_ref, phik_ref, vt_ref, kvt_ref,
            xin_ref, xn_ref, wqkv_ref, wo_ref, w1t_ref, w2_ref, w_sems, x_sems, o_sems):
    NCT = 3 * D // 128
    wq_copies = [
        pltpu.make_async_copy(wqkv_hbm.at[:, pl.ds(j * 128, 128)],
                              wqkv_ref.at[:, pl.ds(j * 128, 128)], w_sems.at[3 + j])
        for j in range(NCT)
    ]
    x_copies = [
        pltpu.make_async_copy(x_hbm.at[pl.ds(i * T, T), :],
                              xin_ref.at[pl.ds(i * T, T), :], x_sems.at[i])
        for i in range(NT_TILES)
    ]
    wo_copy = pltpu.make_async_copy(wo_hbm, wo_ref, w_sems.at[0])
    w1_copy = pltpu.make_async_copy(w1t_hbm, w1t_ref, w_sems.at[1])
    w2_copy = pltpu.make_async_copy(w2_hbm, w2_ref, w_sems.at[2])
    for c in wq_copies + x_copies + [wo_copy, w1_copy, w2_copy]:
        c.start()

    wv = wphi_ref[...]
    wcat = jnp.concatenate([wv[d] for d in range(DH)], axis=1)
    r640 = lax.broadcasted_iota(jnp.int32, (D, D), 0)
    c640 = lax.broadcasted_iota(jnp.int32, (D, D), 1)
    e_dh = (c640 == (r640 % H) * DH + r640 // H).astype(jnp.bfloat16)
    z = _dot(wcat, e_dh, _NN).astype(jnp.bfloat16)
    z = jnp.concatenate([z, jnp.zeros((32 - DH, D), jnp.bfloat16)], axis=0)

    r32 = lax.broadcasted_iota(jnp.int32, (GW, 32), 0)
    c32 = lax.broadcasted_iota(jnp.int32, (GW, 32), 1)
    sel_f = (c32 == r32 // L).astype(jnp.bfloat16)
    rowg = lax.broadcasted_iota(jnp.int32, (GW, WIN), 0)
    colw = lax.broadcasted_iota(jnp.int32, (GW, WIN), 1)
    gts, perms = [], []
    for g in range(NG):
        w0 = _win0(g)
        col = colw + w0
        head = g * L + rowg % L
        gfull = _dot(sel_f, z[:, w0:w0 + WIN], _NN)
        gts.append(jnp.where(col // DH == head, gfull, 0.0).astype(jnp.bfloat16))
        perms.append((col == head * DH + rowg // L).astype(jnp.bfloat16))

    waited = set()

    def need(part, g):
        for j in (part * (D // 128) + _win0(g) // 128, part * (D // 128) + _win0(g) // 128 + 1):
            if j not in waited:
                waited.add(j)
                wq_copies[j].wait()

    for part, lhs in ((0, gts), (1, gts), (2, perms)):
        for g in range(NG):
            need(part, g)
            w0 = part * D + _win0(g)
            wt_ref[part * D + g * GW:part * D + (g + 1) * GW, :] = _dot(
                lhs[g], wqkv_ref[:, w0:w0 + WIN], _NT).astype(jnp.bfloat16)

    zpad = jnp.zeros((PHI_ROWS - 2 * GW, S), jnp.bfloat16)
    ones_rows = jnp.concatenate(
        [jnp.ones((L, S), jnp.bfloat16), jnp.zeros((V_ROWS - GW - L, S), jnp.bfloat16)], axis=0)
    for g in range(NG):
        phiq_ref[g, 2 * GW:PHI_ROWS, :] = zpad
        phik_ref[g, 2 * GW:PHI_ROWS, :] = zpad
        vt_ref[g, GW:V_ROWS, :] = ones_rows

    def ln_tile(t0):
        xn_ref[pl.ds(t0, TB), :] = _layernorm_bf16(xs_ref[pl.ds(t0, TB), :])

    def a1_work(xn, t0):
        pv = _dot(wt_ref[...], xn, _NT)
        phiq = _hedgehog_features(pv[0:D])
        phik = _hedgehog_features(pv[D:2 * D])
        vt = pv[2 * D:3 * D].reshape(NG, GW, T).astype(jnp.bfloat16)
        for g in range(NG):
            phiq_ref[g, 0:2 * GW, pl.ds(t0, T)] = phiq[g]
            phik_ref[g, 0:2 * GW, pl.ds(t0, T)] = phik[g]
            vt_ref[g, 0:GW, pl.ds(t0, T)] = vt[g]

    def a1_first_step(i, carry):
        t0 = pl.multiple_of(i * T, T)
        pltpu.make_async_copy(x_hbm.at[pl.ds(t0, T), :],
                              xin_ref.at[pl.ds(t0, T), :], x_sems.at[i]).wait()
        a1_work(_layernorm_bf16(xin_ref[pl.ds(t0, T), :].astype(jnp.float32)), t0)
        return carry

    def a1_step(i, carry):
        t0 = pl.multiple_of(i * T, T)
        a1_work(_layernorm_bf16(xs_ref[pl.ds(t0, T), :]), t0)
        return carry

    def a_state():
        r = lax.broadcasted_iota(jnp.int32, (V_ROWS, PHI_ROWS), 0)
        c = lax.broadcasted_iota(jnp.int32, (V_ROWS, PHI_ROWS), 1)
        same_head = (r % L) == (c % L)
        for g in range(NG):
            kv = _dot(vt_ref[g], phik_ref[g], _NT)
            kvt_ref[g] = jnp.where(same_head, kv, 0.0).astype(jnp.bfloat16)

    def a2_work(t0, first=False):
        outs = []
        for g in range(NG):
            nd = _dot(kvt_ref[g], phiq_ref[g, :, pl.ds(t0, T)], _NN)
            inv = 1.0 / (nd[GW:GW + L] + 1e-6)
            o = nd[0:GW].reshape(DH, L, T) * inv[None]
            outs.append(o.reshape(GW, T).astype(jnp.bfloat16))
        ot = jnp.concatenate(outs, axis=0)
        attn = _dot(ot, wop_ref[...], _TN)
        if first:
            xs_ref[pl.ds(t0, T), :] = xin_ref[pl.ds(t0, T), :].astype(jnp.float32) + attn
        else:
            xs_ref[pl.ds(t0, T), :] += attn

    def a2_first_step(i, carry):
        a2_work(pl.multiple_of(i * T, T), first=True)
        return carry

    def a2_step(i, carry):
        a2_work(pl.multiple_of(i * T, T))
        return carry

    def b_work(t0):
        xn = xn_ref[pl.ds(t0, TB), :]
        h = _dot(xn, w1t_ref[...], _NT)
        h = (h * jax.nn.sigmoid(h)).astype(jnp.bfloat16)
        y = _dot(h, w2_ref[...], _NN)
        return xs_ref[pl.ds(t0, TB), :] + y

    def b_step(i, carry):
        t0 = pl.multiple_of(i * TB, TB)
        t1 = pl.multiple_of((i + 1) * TB, TB)
        ln_tile(t1)
        xs_ref[pl.ds(t0, TB), :] = b_work(t0)
        return carry

    def out_copy(i, t0):
        return pltpu.make_async_copy(xin_ref.at[pl.ds(t0, TB), :],
                                     o_hbm.at[pl.ds(t0, TB), :], o_sems.at[i])

    def b_last_step(i, carry):
        t0 = pl.multiple_of(i * TB, TB)
        t1 = pl.multiple_of((i + 1) * TB, TB)
        ln_tile(t1)
        xin_ref[pl.ds(t0, TB), :] = b_work(t0).astype(xin_ref.dtype)
        out_copy(i, t0).start()
        return carry

    NL = NT_TILES - 1
    LAST = NL * T
    NBL = NB_TILES - 1
    BLAST = NBL * TB

    lax.fori_loop(0, NT_TILES, a1_first_step, 0)
    a_state()
    wo_copy.wait()
    for g in range(NG):
        w0 = _win0(g)
        wop_ref[g * GW:(g + 1) * GW, :] = _dot(
            perms[g], wo_ref[w0:w0 + WIN, :], _NN).astype(jnp.bfloat16)
    lax.fori_loop(0, NL, a2_first_step, 0)
    ln_tile(0)
    a2_work(LAST, first=True)
    w1_copy.wait()
    w2_copy.wait()
    lax.fori_loop(0, NBL, b_step, 0)
    xs_ref[BLAST:BLAST + TB, :] = b_work(BLAST)
    lax.fori_loop(0, NT_TILES, a1_step, 0)
    a_state()
    lax.fori_loop(0, NL, a2_step, 0)
    ln_tile(0)
    a2_work(LAST)
    lax.fori_loop(0, NBL, b_last_step, 0)
    HB = TB // 2
    tail_copies = []
    for hh in range(2):
        r0 = BLAST + hh * HB
        xn = xn_ref[r0:r0 + HB, :]
        h = _dot(xn, w1t_ref[...], _NT)
        h = (h * jax.nn.sigmoid(h)).astype(jnp.bfloat16)
        y = _dot(h, w2_ref[...], _NN)
        xin_ref[r0:r0 + HB, :] = (xs_ref[r0:r0 + HB, :] + y).astype(xin_ref.dtype)
        cp = pltpu.make_async_copy(xin_ref.at[pl.ds(r0, HB), :],
                                   o_hbm.at[pl.ds(r0, HB), :], o_sems.at[NBL + hh])
        cp.start()
        tail_copies.append(cp)
    for i in range(NBL):
        out_copy(i, i * TB).wait()
    for cp in tail_copies:
        cp.wait()


@jax.jit
def pallas_interleave_layers__linear_kernel_hedgehog__dense_activation_silu__prompt_kernel(
    A_x: jax.Array,
    A_wqkv: jax.Array,
    A_w_phi: jax.Array,
    A_wo: jax.Array,
    B_x: jax.Array,
    B_w1: jax.Array,
    B_w2: jax.Array,
):
    del B_x
    assert A_x.shape == (1, S, D) and A_wqkv.shape == (D, 3 * D) and A_w_phi.shape == (H, DH, DH)
    assert A_wo.shape == (D, D) and B_w1.shape == (D, F) and B_w2.shape == (F, D)
    x = A_x.reshape(S, D)
    wphi = A_w_phi.transpose(1, 2, 0)

    out = pl.pallas_call(
        _kernel,
        out_shape=jax.ShapeDtypeStruct((S, D), A_x.dtype),
        in_specs=[
            pl.BlockSpec(memory_space=pl.ANY),
            pl.BlockSpec(memory_space=pl.ANY),
            pl.BlockSpec(memory_space=pltpu.VMEM),
            pl.BlockSpec(memory_space=pl.ANY),
            pl.BlockSpec(memory_space=pl.ANY),
            pl.BlockSpec(memory_space=pl.ANY),
        ],
        out_specs=pl.BlockSpec(memory_space=pl.ANY),
        scratch_shapes=[
            pltpu.VMEM((S, D), jnp.float32),
            pltpu.VMEM((3 * D, D), jnp.bfloat16),
            pltpu.VMEM((D, D), jnp.bfloat16),
            pltpu.VMEM((NG, PHI_ROWS, S), jnp.bfloat16),
            pltpu.VMEM((NG, PHI_ROWS, S), jnp.bfloat16),
            pltpu.VMEM((NG, V_ROWS, S), jnp.bfloat16),
            pltpu.VMEM((NG, V_ROWS, PHI_ROWS), jnp.bfloat16),
            pltpu.VMEM((S, D), jnp.bfloat16),
            pltpu.VMEM((S, D), jnp.bfloat16),
            pltpu.VMEM((D, 3 * D), jnp.bfloat16),
            pltpu.VMEM((D, D), jnp.bfloat16),
            pltpu.VMEM((F, D), jnp.bfloat16),
            pltpu.VMEM((F, D), jnp.bfloat16),
            pltpu.SemaphoreType.DMA((3 + 3 * D // 128,)),
            pltpu.SemaphoreType.DMA((NT_TILES,)),
            pltpu.SemaphoreType.DMA((NB_TILES + 1,)),
        ],
        compiler_params=pltpu.CompilerParams(vmem_limit_bytes=100 * 1024 * 1024),
    )(x, A_wqkv, wphi, A_wo, B_w1.T, B_w2)
    return out.reshape(1, S, D)
```
